```python
import os as _os
_os.environ.setdefault("JAX_PLATFORMS", "cpu")
import jax
import jax.numpy as jnp

def _softmax(x, axis=-1):
    return jax.nn.softmax(x, axis=axis)
def _gelu(x):
    return jax.nn.gelu(x, approximate=True)
def _silu(x):
    return jax.nn.silu(x)
def _sigmoid(x):
    return jax.nn.sigmoid(x)
def _layernorm(x, axis=-1, eps=1e-5):
    m = jnp.mean(x, axis=axis, keepdims=True)
    v = jnp.var(x, axis=axis, keepdims=True)
    return (x - m) / jnp.sqrt(v + eps)
def _scatter_add(tgt, idx, src, axis=0):
    return tgt.at[idx].add(src)
def _segment_sum(src, seg, n):
    return jax.ops.segment_sum(src, seg, n)
class _Rng:
    def __init__(self, key):
        self._k = key
    def _next(self):
        self._k, sub = jax.random.split(self._k)
        return sub
    def normal(self, shape):
        return jax.random.normal(self._next(), shape, dtype=jnp.bfloat16)
    def randint(self, lo, hi, shape):
        return jax.random.randint(self._next(), shape, lo, hi, dtype=jnp.int32)
    def uniform(self, shape, lo=0.0, hi=1.0):
        return jax.random.uniform(self._next(), shape, jnp.bfloat16, lo, hi)
    def permutation(self, n):
        return jax.random.permutation(self._next(), n)


kernel_name = 'concat_heads__softmax_full_mha__grouped_kv_mqa__prompt'

def setup_inputs():
    _rng = _Rng(jax.random.key(int.from_bytes(__import__("os").urandom(4), "little")))
    _w = (lambda a: (lambda t: t.astype(jnp.bfloat16) if jnp.issubdtype(t.dtype, jnp.floating) else t)(jnp.asarray(a)))
    def _A_setup():
        B, S, D = 1, 2048, 640
        return {
            "x": _w((lambda *s: _rng.normal(s) * 0.1)(B, S, D)),
            "wqkv": _w((lambda *s: _rng.normal(s) * 0.1)(D, 3 * D)),
            "wo": _w((lambda *s: _rng.normal(s) * 0.05)(D, D)),
        }
    _A_in = _A_setup()

    def _B_setup():
        B, S, D, H = 1, 2048, 640, 32
        Dh = D // H
        return {
            "x": _w((lambda *s: _rng.normal(s) * 0.05)(B, S, D)),
            "wq": _w((lambda *s: _rng.normal(s) * 0.4)(D, H * Dh)),
            "wk": _w((lambda *s: _rng.normal(s) * 0.4)(D, Dh)),
            "wv": _w((lambda *s: _rng.normal(s) * 0.05)(D, Dh)),
            "wo": _w((lambda *s: _rng.normal(s) * 0.05)(H * Dh, D)),
        }
    _B_in = _B_setup()

    return {
        "A_x": _A_in["x"],
        "A_wqkv": _A_in["wqkv"],
        "A_wo": _A_in["wo"],
        "B_x": _B_in["x"],
        "B_wq": _B_in["wq"],
        "B_wk": _B_in["wk"],
        "B_wv": _B_in["wv"],
        "B_wo": _B_in["wo"],
    }

def reference(A_x, A_wqkv, A_wo, B_x, B_wq, B_wk, B_wv, B_wo):
    def _A_ref(x, wqkv, wo):
        B, S, D = x.shape
        H = 32; Dh = D // H
        qkv = (lambda x, *d: x.transpose(*d))((x @ wqkv).reshape(B, S, 3, H, Dh), 2, 0, 3, 1, 4)
        q, k, v = qkv[0], qkv[1], qkv[2]
        scale = Dh ** -0.5
        scores = jnp.einsum("bhqd,bhkd->bhqk", q, k) * scale
        p = _softmax(scores, axis=-1)
        o = jnp.einsum("bhqk,bhkd->bhqd", p, v)
        return (lambda x, *d: x.transpose(*d))(o, 0, 2, 1, 3).reshape(B, S, D) @ wo

    def _B_ref(x, wq, wk, wv, wo):
        B, S, D = x.shape
        H = 32
        Dh = D // H
        q = (lambda x, *d: x.transpose(*d))((x @ wq).reshape(B, S, H, Dh), 0, 2, 1, 3)
        k = x @ wk
        v = x @ wv
        scores = jnp.einsum("bhqd,bkd->bhqk", q, k) * (Dh ** -0.5)
        p = _softmax(scores, axis=-1)
        o = jnp.einsum("bhqk,bkd->bhqd", p, v)
        return (lambda x, *d: x.transpose(*d))(o, 0, 2, 1, 3).reshape(B, S, H * Dh) @ wo

    a = _A_ref(A_x, A_wqkv, A_wo)
    b = _B_ref(B_x, B_wq, B_wk, B_wv, B_wo)
    return jnp.concatenate([a, b], axis=-1)
```

```python
import functools, math
import jax
import jax.numpy as jnp
from jax import lax
import jax.experimental.pallas as pl
import jax.experimental.pallas.tpu as pltpu

S = 2048
D = 640
H = 32
DH = 20
VR = 24
LOG2E = 1.4426950408889634
F32 = jnp.float32
BF16 = jnp.bfloat16
NT = (((1,), (1,)), ((), ()))
TN = (((0,), (0,)), ((), ()))


def make_kernel(TQ=512, CK=128, U=2, PBF16=True):
    NQS = S // TQ
    RB = TQ
    NSUP = H * NQS
    qscale = (DH ** -0.5) * LOG2E

    def kernel(ax_ref, wqkv_ref, awo_ref, bx_ref, bwq_ref, bwk_ref, bwv_ref, bwo_ref,
               o_ref,
               wTa, wTb, wkvb, kbuf, qT, vT, sA, sB, oT):
        for c in range(5):
            wTa[pl.ds(c * 128, 128), :] = wqkv_ref[:, pl.ds(c * 128, 128)].T
            wTa[pl.ds(D + c * 128, 128), :] = wqkv_ref[:, pl.ds(2 * D + c * 128, 128)].T
            wTb[pl.ds(c * 128, 128), :] = bwq_ref[:, pl.ds(c * 128, 128)].T
        wkvb[...] = jnp.zeros(wkvb.shape, wkvb.dtype)
        wkvb[:, pl.ds(0, DH)] = bwk_ref[...]
        wkvb[:, pl.ds(32, DH)] = bwv_ref[...]

        def proj(r, carry):
            r0 = pl.multiple_of(r * RB, RB)
            lane = lax.broadcasted_iota(jnp.int32, (256, 128), 1)
            row = lax.broadcasted_iota(jnp.int32, (VR, RB), 0)
            for sub in range(RB // 256):
                rows = pl.ds(r0 + sub * 256, 256)
                xa = ax_ref[rows, :]
                ka = jnp.dot(xa, wqkv_ref[:, pl.ds(D, D)], preferred_element_type=F32)
                ws = [ka[:, w * 128:(w + 1) * 128] for w in range(5)]
                for w in range(5):
                    kbuf[w, rows, :] = ws[w].astype(BF16)
                for w in range(4):
                    kbuf[5 + w, rows, :] = jnp.where(lane >= 64, ws[w], ws[w + 1]).astype(BF16)
                xb = bx_ref[rows, :]
                kvb = jnp.dot(xb, wkvb[...], preferred_element_type=F32)
                kvb2 = pltpu.roll(kvb, 4, 1)
                kbuf[9, rows, :] = kvb.astype(BF16)
                kbuf[10, rows, :] = kvb2.astype(BF16)
                rw = lax.broadcasted_iota(jnp.int32, (VR, 256), 0)
                vT[H, r, :, pl.ds(sub * 256, 256)] = jnp.where(rw == DH, 1.0, kvb.T[32:32 + VR, :])
                vT[H + 1, r, :, pl.ds(sub * 256, 256)] = jnp.where(rw == 0, 1.0, kvb2.T[32:32 + VR, :])
            xa = ax_ref[pl.ds(r0, RB), :]
            xb = bx_ref[pl.ds(r0, RB), :]
            for c in range(5):
                q = lax.dot_general(wTa[pl.ds(c * 128, 128), :], xa, NT, preferred_element_type=F32)
                qT[0, r, pl.ds(c * 128, 128), :] = (q * qscale).astype(BF16).astype(F32)
                q = lax.dot_general(wTb[pl.ds(c * 128, 128), :], xb, NT, preferred_element_type=F32)
                qT[1, r, pl.ds(c * 128, 128), :] = (q * qscale).astype(BF16).astype(F32)
            for c in range(4):
                v = lax.dot_general(wTa[pl.ds(D + c * 160, 160), :], xa, NT, preferred_element_type=F32)
                for j in range(4):
                    e = v[40 * j:40 * j + VR, :]
                    o = v[40 * j + 16:40 * j + 16 + VR, :]
                    vT[c * 8 + 2 * j, r] = jnp.where(row == DH, 1.0, e)
                    vT[c * 8 + 2 * j + 1, r] = jnp.where(row == 0, 1.0, o)
            return carry

        lax.fori_loop(0, S // RB, proj, 0)

        row128 = lax.broadcasted_iota(jnp.int32, (128, TQ), 0)

        def weights_a(h, qs):
            start = DH * h
            w = start // 128
            lo = start - w * 128
            w1 = jnp.minimum(w + 1, 4)
            q0 = qT[0, qs, pl.ds(pl.multiple_of(w * 128, 128), 128), :]
            q1 = qT[0, qs, pl.ds(pl.multiple_of(w1 * 128, 128), 128), :]
            m0 = jnp.logical_and(row128 >= lo, row128 < lo + DH)
            m1 = row128 < lo + DH - 128
            wts = jnp.where(m0, q0, jnp.where(m1, q1, 0.0)).astype(BF16)
            kidx = jnp.where(lo + DH > 128, 5 + w, w)
            return wts, kidx

        def weights_b(h, qs):
            par = h % 2
            start = pl.multiple_of(DH * h - 4 * par, 8)
            wts = qT[1, qs, pl.ds(start, VR), :]
            return wts, 9 + par

        def super_stage(u_qk, u_pv, mA, mB):
            do_qk = u_qk is not None
            do_pv = u_pv is not None
            if do_qk:
                h, qs = u_qk // NQS, u_qk % NQS
                wa, ka_i = weights_a(h, qs)
                wb, kb_i = weights_b(h, qs)
                rA = rB = None
            if do_pv:
                hp, qp = u_pv // NQS, u_pv % NQS
                par = hp % 2
                accA = jnp.zeros((VR, TQ), F32)
                accB = jnp.zeros((VR, TQ), F32)
            for c in range(S // CK):
                rows = pl.ds(c * CK, CK)
                vc, vo = (c * CK) // RB, (c * CK) % RB
                if do_pv:
                    p = jnp.exp2(sA[rows, :] - mA)
                    if PBF16:
                        p = p.astype(BF16)
                    accA = accA + jnp.dot(vT[hp, vc, :, pl.ds(vo, CK)], p, preferred_element_type=F32)
                if do_qk:
                    s = jnp.dot(kbuf[ka_i, rows, :], wa, preferred_element_type=F32)
                    sA[rows, :] = s
                    mc = jnp.max(s.reshape(CK // 8, 8, TQ), axis=0)
                    rA = mc if rA is None else jnp.maximum(rA, mc)
                if do_pv:
                    p = jnp.exp2(sB[rows, :] - mB)
                    if PBF16:
                        p = p.astype(BF16)
                    accB = accB + jnp.dot(vT[H + par, vc, :, pl.ds(vo, CK)], p, preferred_element_type=F32)
                if do_qk:
                    s = jnp.dot(kbuf[kb_i, rows, pl.ds(0, VR)], wb, preferred_element_type=F32)
                    sB[rows, :] = s
                    mc = jnp.max(s.reshape(CK // 8, 8, TQ), axis=0)
                    rB = mc if rB is None else jnp.maximum(rB, mc)
            if do_pv:
                for b, acc in ((0, accA), (1, accB)):
                    l = jnp.where(par == 1, acc[0:1, :], acc[DH:DH + 1, :])
                    oT[b, hp, qp] = acc * (1.0 / l)
            if do_qk:
                return (jnp.max(rA, axis=0, keepdims=True), jnp.max(rB, axis=0, keepdims=True))
            return None

        ms = super_stage(jnp.int32(0), None, None, None)

        def body(j, ms):
            for t in range(U):
                u = j * U + t
                ms = super_stage(jnp.minimum(u + 1, NSUP - 1), u, *ms)
            return ms

        lax.fori_loop(0, NSUP // U, body, ms)

        def outp(qs, carry):
            r8 = lax.broadcasted_iota(jnp.int32, (8, TQ), 0)
            for b, wo_ref in enumerate((awo_ref, bwo_ref)):
                parts = []
                for j in range(H // 2):
                    e = oT[b, 2 * j, qs]
                    o = oT[b, 2 * j + 1, qs]
                    parts += [e[0:16], jnp.where(r8 < 4, e[16:24], o[0:8]), o[8:24]]
                ot = jnp.concatenate(parts, axis=0).astype(BF16)
                out = lax.dot_general(ot, wo_ref[...], TN, preferred_element_type=F32)
                o_ref[pl.ds(pl.multiple_of(qs * TQ, TQ), TQ), pl.ds(b * D, D)] = out.astype(o_ref.dtype)
            return carry

        lax.fori_loop(0, NQS, outp, 0)

    @jax.jit
    def fn(A_x, A_wqkv, A_wo, B_x, B_wq, B_wk, B_wv, B_wo):
        args = (A_x.reshape(S, D), A_wqkv, A_wo, B_x.reshape(S, D), B_wq, B_wk, B_wv, B_wo)
        out = pl.pallas_call(
            kernel,
            out_shape=jax.ShapeDtypeStruct((S, 2 * D), BF16),
            scratch_shapes=[
                pltpu.VMEM((2 * D, D), BF16),
                pltpu.VMEM((D, D), BF16),
                pltpu.VMEM((D, 128), BF16),
                pltpu.VMEM((11, S, 128), BF16),
                pltpu.VMEM((2, NQS, D, TQ), F32),
                pltpu.VMEM((H + 2, S // RB, VR, RB), F32),
                pltpu.VMEM((S, TQ), F32),
                pltpu.VMEM((S, TQ), F32),
                pltpu.VMEM((2, H, NQS, VR, TQ), F32),
            ],
            compiler_params=pltpu.CompilerParams(vmem_limit_bytes=100 * 1024 * 1024),
            name="attn",
        )(*args)
        return out.reshape(1, S, 2 * D)

    return fn


_fn = make_kernel()


@jax.jit
def pallas_concat_heads__softmax_full_mha__grouped_kv_mqa__prompt_kernel(
    A_x, A_wqkv, A_wo, B_x, B_wq, B_wk, B_wv, B_wo,
):
    return _fn(A_x, A_wqkv, A_wo, B_x, B_wq, B_wk, B_wv, B_wo)
```

```python
import jax
import jax.numpy as jnp
from jax import lax
import jax.experimental.pallas as pl
import jax.experimental.pallas.tpu as pltpu

S = 2048
D = 640
H = 32
DH = 20
VR = 24
F32 = jnp.float32
BF16 = jnp.bfloat16
U32 = jnp.uint32
NT = (((1,), (1,)), ((), ()))
TN = (((0,), (0,)), ((), ()))
ONE2 = 0x3F803F80
QSCALE = (DH ** -0.5) * 1.4426950408889634
INFL = 1.0 + 2.0 ** -6
THR = 2.0 ** -40

TQ = 512
CK = 128
NQS = S // TQ
NCH = S // CK
NL = TQ // 128
NITEM = (H // 2) * NQS
NS = 4
NV = [(48, 32, 32, 32)[c % 4] for c in range(NCH)]
SHIFT = (16, 48)
TAIL = 64
GV = max(NV) // 8
EK = -(-GV // NL)
EH = S // 16 // NL
P_QBC = 0
P_PV = P_QBC + NS * (DH + 1)
P_WST = P_PV + NS * NCH * GV
P_KBC = P_WST + NS * 2 * 3
P_KB = P_KBC + NCH * DH * EK
P_VB = P_KB + 2 * EH
P_KA = P_VB + 2 * 3 * NQS
P_VA = P_KA + 2 * EH
P_DEF = P_VA + 2 * 3 * NQS
P_ACC = P_DEF + 16
P_END = P_ACC + 3
AX, BX = 8, 8 + NQS


def _f2u(x):
    return lax.bitcast_convert_type(x, U32)


def _u2f(x):
    return lax.bitcast_convert_type(x, F32)


def _lanes(lt):
    return pl.ds(lt * 128, 128)


def _iota(shape, dim):
    return lax.broadcasted_iota(jnp.int32, shape, dim)


def _rev8(x):
    return jnp.concatenate([x[c * CK + g * 8:c * CK + g * 8 + 8] for c in range(x.shape[0] // CK)
                            for g in range(CK // 8 - 1, -1, -1)], axis=0)


def _gate_at(events, frac, tail=TAIL):
    x = frac * (sum(e.shape[0] // 8 * NL * w for e, w in events) - tail)
    for e, w in events:
        per = e.shape[0] // 8 * NL
        if x < per * w:
            vi = min(int(x / w), per - 1)
            g, lt = (vi // NL) * 8, vi % NL
            return e[g:g + 8, lt * 128:(lt + 1) * 128]
        x -= per * w


def _kernel(ax_hbm, wqkv_hbm, awo_hbm, bx_hbm, bwq_hbm, bwkT_hbm, bwvT_hbm, bwo_hbm,
            o_hbm,
            ax, bx, wka, wsrc, wkT, wvT, wo, obuf,
            wT, wkvT, kh, qT, vT, oT, pool, kmax, mt, kw, sfb, zref, isem, osem):
    zref[0] = 0
    cp = pltpu.make_async_copy

    def x_copy(hbm, buf, base, r):
        rows = pl.ds(pl.multiple_of(r * TQ, TQ), TQ)
        return cp(hbm.at[rows, :], buf.at[rows, :], isem.at[base + r])

    c_wka = cp(wqkv_hbm.at[:, pl.ds(D, D)], wka, isem.at[0])
    c_ws = [cp(wqkv_hbm.at[:, pl.ds(0, D)], wsrc.at[:, pl.ds(0, D)], isem.at[1]),
            cp(wqkv_hbm.at[:, pl.ds(2 * D, D)], wsrc.at[:, pl.ds(D, D)], isem.at[2]),
            cp(bwq_hbm, wsrc.at[:, pl.ds(2 * D, D)], isem.at[3])]
    c_small = [cp(bwkT_hbm, wkT, isem.at[4]), cp(bwvT_hbm, wvT, isem.at[5])]
    c_wo = [cp(awo_hbm, wo.at[0], isem.at[6]), cp(bwo_hbm, wo.at[1], isem.at[7])]

    c_wka.start()
    for r in range(NQS - 1):
        x_copy(ax_hbm, ax, AX, r).start()
    for c in c_ws:
        c.start()
    x_copy(ax_hbm, ax, AX, NQS - 1).start()
    for c in c_small:
        c.start()
    for r in range(NQS):
        x_copy(bx_hbm, bx, BX, r).start()
    for c in c_wo:
        c.start()

    def k_proj(r, kma):
        x_copy(ax_hbm, ax, AX, r).wait()
        for sub in range(TQ // 256):
            rows = pl.ds(pl.multiple_of(r * TQ, TQ) + sub * 256, 256)
            prow = pl.ds(pl.multiple_of(r * (TQ // 2), TQ // 2) + sub * 128, 128)
            ka = jnp.dot(ax[rows, :], wka[...], preferred_element_type=F32)
            kma = jnp.maximum(kma, jnp.max(jnp.abs(ka).reshape(32, 8, D), axis=0))
            ka = _rev8(ka)
            for w in range(5):
                kw[w, prow, :] = pltpu.bitcast(ka[:, w * 128:(w + 1) * 128].astype(BF16), U32)
        return kma

    c_wka.wait()
    kma = lax.fori_loop(0, NQS - 1, k_proj, jnp.zeros((8, D), F32))
    for c in c_ws:
        c.wait()
    for c in c_small:
        c.wait()
    kma = k_proj(NQS - 1, kma)
    for i in range(15):
        wT[pl.ds(i * 128, 128), :] = wsrc[:, pl.ds(i * 128, 128)].T
    wkvT[...] = jnp.zeros(wkvT.shape, wkvT.dtype)
    wkvT[pl.ds(0, DH), :] = wkT[...]
    wkvT[pl.ds(32, DH), :] = wvT[...]

    hrow, hcol = _iota((H, D), 0), _iota((H, D), 1)
    inhead = jnp.logical_and(hcol >= hrow * DH, hcol < hrow * DH + DH)
    kmax[0] = jnp.where(inhead, jnp.max(kma, axis=0, keepdims=True) * INFL, 0.0)

    def bound(b, r):
        qa = jnp.abs(qT[b, r].reshape(D, TQ))
        bd = jnp.dot(kmax[b], qa, preferred_element_type=F32)
        nb = (-(bd * INFL)).astype(BF16).astype(F32)
        for h in range(H):
            mt[b, r, h] = jnp.broadcast_to(nb[h:h + 1, :], (8, TQ))

    def proj(r, kmb):
        x_copy(bx_hbm, bx, BX, r).wait()
        r0 = pl.multiple_of(r * TQ, TQ)
        row = _iota((VR, TQ), 0)
        xs = (ax[pl.ds(r0, TQ), :], bx[pl.ds(r0, TQ), :])

        lane = _iota((128, 128), 1)
        rw = _iota((VR, 256), 0)
        for sub in range(TQ // 256):
            rows = pl.ds(r0 + sub * 256, 256)
            kvb = lax.dot_general(bx[rows, :], wkvT[...], NT, preferred_element_type=F32)
            kmb = jnp.maximum(kmb, jnp.max(jnp.abs(kvb).reshape(32, 8, 128), axis=0))
            kvb2 = pltpu.roll(kvb, 4, 1)
            k1 = pltpu.bitcast(_rev8(kvb).astype(BF16), U32)
            k2 = pltpu.bitcast(_rev8(kvb2).astype(BF16), U32)
            k1 = jnp.where(lane == DH, jnp.uint32(ONE2), k1)
            k2 = jnp.where(lane == 0, jnp.uint32(ONE2), k2)
            e0 = r * (EH // NQS) + sub * (16 // NL)
            for par, kk in ((0, k1), (1, k2)):
                for t in range(16):
                    pool[P_KB + par * EH + e0 + t // NL, :, _lanes(t % NL)] = kk[t * 8:(t + 1) * 8]
            for cc in range(256 // CK):
                ci = r * (TQ // CK) + sub * (256 // CK) + cc
                gv = NV[sub * (256 // CK) + cc] // 8
                kr = kvb[cc * CK:cc * CK + gv * 8, :].astype(BF16).astype(F32)
                for d in range(DH):
                    kb = _f2u(jnp.broadcast_to(kr[:, d:d + 1], (gv * 8, 128)))
                    for g in range(gv):
                        pool[P_KBC + (ci * EK + g // NL) * DH + d, :, _lanes(g % NL)] = kb[g * 8:(g + 1) * 8]
            v1 = _f2u(jnp.where(rw == DH, 1.0, kvb.T[32:32 + VR, :]))
            v2 = _f2u(jnp.where(rw == 0, 1.0, kvb2.T[32:32 + VR, :]))
            for par, vv in ((0, v1), (1, v2)):
                for t in range(3):
                    pool[P_VB + (par * 3 + t) * NQS + r, :, pl.ds(sub * 256, 256)] = vv[t * 8:(t + 1) * 8]

        def q_proj(b):
            for c in range(5):
                q = lax.dot_general(wT[pl.ds(2 * D * b + c * 128, 128), :], xs[b], NT,
                                    preferred_element_type=F32)
                q = (q * QSCALE).astype(BF16).astype(F32)
                qT[b, r, pl.ds(c * 16, 16)] = q.reshape(16, 8, TQ)

        def v_proj(c):
            v = lax.dot_general(wT[pl.ds(D + c * 160, 160), :], xs[0], NT, preferred_element_type=F32)
            for j in range(4):
                e = v[40 * j:40 * j + VR, :]
                o = v[40 * j + 16:40 * j + 16 + VR, :]
                vT[c * 8 + 2 * j, r] = jnp.where(row == DH, 1.0, e)
                vT[c * 8 + 2 * j + 1, r] = jnp.where(row == 0, 1.0, o)

        q_proj(0)
        v_proj(0)
        v_proj(1)
        bound(0, r)
        v_proj(2)
        v_proj(3)
        q_proj(1)
        lane = _iota((64, 128), 1)
        for sub in range(TQ // 128):
            prow = pl.ds(pl.multiple_of(r * (TQ // 2), TQ // 2) + sub * 64, 64)
            ws = [kw[w, prow, :] for w in range(5)]
            for h in range(H):
                w, lo = divmod(DH * h, 128)
                src = ws[w] if lo + DH <= 128 else jnp.where(lane >= 64, ws[w], ws[w + 1])
                off = 4 * (h % 2)
                sh = (128 - lo + off) % 128
                if sh:
                    src = pltpu.roll(src, sh, 1)
                keep = (lane >= off) if off else (lane < DH)
                fill = jnp.where(lane == (0 if off else DH), jnp.uint32(ONE2), jnp.uint32(0))
                kh[h, prow, :] = jnp.where(keep, src, fill)
        return kmb

    kmb = lax.fori_loop(0, NQS, proj, jnp.zeros((8, 128), F32))

    trow, tcol = _iota((128, D), 0), _iota((128, D), 1)
    sel = jnp.zeros((128, D), F32)
    for h in range(H):
        sel = jnp.where(jnp.logical_and(tcol - h * DH == trow, trow < DH), 1.0, sel)
    kmb_up = (jnp.max(kmb, axis=0, keepdims=True) * INFL).astype(BF16).astype(F32)
    kmb_up = jnp.where(_iota((8, 128), 1) < DH, jnp.broadcast_to(kmb_up, (8, 128)), 0.0)
    kmb_t = jnp.dot(kmb_up, sel, preferred_element_type=F32)[0:1, :]
    kmax[1] = jnp.where(inhead, kmb_t, 0.0)
    for r in range(NQS):
        bound(1, r)

    r8 = _iota((8, TQ), 0)

    def q_window(b, it, par):
        j, qs = it // NQS, it % NQS
        w = qT[b, qs, pl.ds(5 * j + 2 * par, 3)]
        nb = mt[b, qs, 2 * j + par]
        if par:
            return jnp.concatenate([jnp.where(r8 == 0, nb, w[0]), w[1], w[2]], axis=0)
        return jnp.concatenate([w[0], w[1], jnp.where(r8 == 4, nb, w[2])], axis=0)

    def build_qbc(it, par, slot, events):
        wb = q_window(1, it, par)
        never = zref[0] != 0
        n = 0
        for t in range(3):
            for lt in range(NL):
                blk = wb[t * 8:(t + 1) * 8, lt * 128:(lt + 1) * 128]
                if events is not None:
                    blk = jnp.where(never, _gate_at(events, (n + 0.5) / (3 * NL + 1)), blk)
                n += 1
                for rr in range(8):
                    d = t * 8 + rr - 4 * par
                    if t * 8 + rr == (0 if par else DH):
                        d = DH
                    elif not 0 <= d < DH:
                        continue
                    v = jnp.broadcast_to(blk[rr:rr + 1, :], (8, 128))
                    pool[P_QBC + slot * (DH + 1) + d, :, _lanes(lt)] = _f2u(v)

    def vpu_scores(pair, chunks, events, tail):
        never = zref[0] != 0
        strips = [(c, g) for c in chunks for g in range(NV[c] // 8)]
        nsteps = len(strips) * DH
        for jb, (c, g) in enumerate(strips):
            gates = jnp.concatenate([_gate_at(events, (jb * DH + d) / nsteps, tail) for d in range(DH)], axis=0)
            kb = _u2f(pool[pl.ds(P_KBC + (c * EK + g // NL) * DH, DH), :, _lanes(g % NL)])
            kb = jnp.where(never, gates.reshape(DH, 8, 128), kb)
            kb = jnp.concatenate([kb] * NL, axis=2)
            for slot in (2 * pair, 2 * pair + 1):
                qi = P_QBC + slot * (DH + 1)
                s = jnp.sum(kb * _u2f(pool[pl.ds(qi, DH)]), axis=0) + _u2f(pool[qi + DH])
                pool[P_PV + (slot * NCH + c) * GV + g] = _f2u(jnp.exp2(s))

    def pool_vt(base, par, c):
        vc, vo = divmod(c * CK, TQ)
        return _u2f(jnp.concatenate([pool[base + (par * 3 + t) * NQS + vc, :, pl.ds(vo, CK)]
                                     for t in range(3)], axis=0))

    def finish(acc, b, it, par, ok):
        lr = 0 if par else DH
        l = acc[lr:lr + 1, :]
        oT[b, 2 * (it // NQS) + par, it % NQS] = acc * (1.0 / l)
        return jnp.where(l >= THR, ok, 0.0)

    class Stage:
        def __init__(self, b, slot, it, events):
            self.b, self.par, self.slot, self.it, self.events = b, slot % 2, slot, it, events
            self.nv = NV if b == 1 else [0] * NCH
            self.head = 2 * (it // NQS) + self.par
            self.groups = [c * 8 + g for c in range(NCH) for g in range((CK - self.nv[c]) // 16)]
            self.pos = 0
            self.p8 = {}
            self.last = False
            self.w0 = P_WST + (slot * 2 + b) * 3
            pool[pl.ds(self.w0, 3)] = _f2u(q_window(b, it, self.par)).reshape(3, 8, TQ)

        def qk(self, c):
            end = sum((CK - self.nv[i]) // 16 for i in range(c + 1)) + SHIFT[self.b] // 16
            gs = self.groups[self.pos:min(end, len(self.groups))]
            self.pos += len(gs)
            if self.b == 1 or self.slot >= 2:
                base = (P_KB if self.b == 1 else P_KA) + self.par * EH
                parts = [pool[base + g // NL, :, _lanes(g % NL)] for g in gs]
            else:
                parts = [kh[self.head, pl.ds(g * 8, 8), :] for g in gs]
                for g, pt in zip(gs, parts):
                    pool[P_KA + self.par * EH + g // NL, :, _lanes(g % NL)] = pt
            kc = pltpu.bitcast(jnp.concatenate(parts, axis=0) if len(parts) > 1 else parts[0], BF16)
            wq = _u2f(pool[pl.ds(self.w0, 3)]).reshape(VR, TQ)
            s = jnp.dot(kc[:, :VR], wq, preferred_element_type=F32)
            nm = S - sum(self.nv)
            self.events.append((s, ((nm + VR * NCH) / nm) / ((CK + VR) / CK)))
            p = jnp.exp2(s)
            for i, g in enumerate(gs):
                self.p8[2 * g] = p[16 * i:16 * i + 8]
                self.p8[2 * g + 1] = p[16 * i + 8:16 * i + 16]

        def pv(self, c, ok):
            b, par, nv = self.b, self.par, self.nv[c]
            parts = []
            if nv:
                parts.append(_u2f(pool[pl.ds(P_PV + (self.slot * NCH + c) * GV, nv // 8)]).reshape(nv, TQ))
            for g in range(nv // 8, CK // 8):
                parts.append(self.p8.pop(c * 16 + 15 - g))
            p = jnp.concatenate(parts, axis=0)
            if self.last and c == NCH - 1:
                pool[pl.ds(P_DEF, 16)] = _f2u(p).reshape(16, 8, TQ)
                return ok
            if b == 1 or self.slot >= 2:
                vt = pool_vt(P_VB if b == 1 else P_VA, par, c)
            else:
                vc, vo = divmod(c * CK, TQ)
                vt = vT[self.head, vc, :, pl.ds(vo, CK)]
                for t in range(3):
                    pool[P_VA + (par * 3 + t) * NQS + vc, :, pl.ds(vo, CK)] = _f2u(vt[t * 8:(t + 1) * 8])
            acc = jnp.dot(vt, p, preferred_element_type=F32)
            if c > 0:
                acc = _u2f(pool[pl.ds(P_ACC, 3)]).reshape(VR, TQ) + acc
            if c < NCH - 1:
                pool[pl.ds(P_ACC, 3)] = _f2u(acc).reshape(3, 8, TQ)
                return ok
            return finish(acc, b, self.it, par, ok)

    def finish_deferred(it, ok):
        acc = _u2f(pool[pl.ds(P_ACC, 3)]).reshape(VR, TQ)
        p = _u2f(pool[pl.ds(P_DEF, 16)]).reshape(CK, TQ)
        acc = acc + jnp.dot(pool_vt(P_VA, 1, NCH - 1), p, preferred_element_type=F32)
        return finish(acc, 0, it, 1, ok)

    def body(i, ok):
        ok = finish_deferred(jnp.maximum(i, 1) * 2 - 1, ok)
        evs = [[] for _ in range(NS)]
        st = []
        for k in range(NS):
            st += [Stage(1, k, i * 2 + k // 2, evs[k]), Stage(0, k, i * 2 + k // 2, evs[k])]
        st[-1].last = True
        slots = [(s, c) for s in st for c in range(NCH)]
        for n in range(len(slots) + 1):
            if n == 3 * NCH:
                vpu_scores(1, range(NCH // 2, NCH), evs[0], 0)
            if n < len(slots):
                slots[n][0].qk(slots[n][1])
                if slots[n][1] == NCH - 1 and n + 1 < len(slots):
                    slots[n + 1][0].qk(-1)
            if n >= 1:
                s, c = slots[n - 1]
                ok = s.pv(c, ok)
        itn = jnp.minimum(i + 1, NITEM // 2 - 1) * 2
        h0 = len(evs[0]) // 2
        build_qbc(itn, 0, 0, evs[0][:h0])
        build_qbc(itn, 1, 1, evs[0][h0:])
        vpu_scores(0, range(NCH), evs[1] + evs[2], 0)
        build_qbc(itn + 1, 0, 2, evs[1])
        build_qbc(itn + 1, 1, 3, evs[2])
        vpu_scores(1, range(NCH // 2), evs[3], TAIL)
        return ok

    for k in range(NS):
        wq = q_window(1, jnp.int32(k // 2), k % 2)
        base = P_KB + (k % 2) * EH
        for c4 in range(NCH // 4 if k < 2 else NCH // 8):
            gl = [c * 8 + 8 - NV[c] // 16 + i for c in range(c4 * 4, c4 * 4 + 4) for i in range(NV[c] // 16)]
            kc = jnp.concatenate([pool[base + g // NL, :, _lanes(g % NL)] for g in gl], axis=0)
            pp = _f2u(jnp.exp2(jnp.dot(pltpu.bitcast(kc, BF16)[:, :VR], wq, preferred_element_type=F32)))
            for i, g in enumerate(gl):
                for hf in range(2):
                    c, st8 = g // 8, (g % 8) * 2 + hf
                    pool[P_PV + (k * NCH + c) * GV + 15 - st8] = pp[16 * i + 8 * hf:16 * i + 8 * hf + 8]
    build_qbc(jnp.int32(1), 0, 2, None)
    build_qbc(jnp.int32(1), 1, 3, None)
    pool[pl.ds(P_DEF, 19)] = _f2u(jnp.ones((19, 8, TQ), F32))
    for t in range(3):
        pool[P_VA + (3 + t) * NQS + NQS - 1] = jnp.zeros((8, TQ), U32)

    ok = lax.fori_loop(0, NITEM // 2, body, jnp.ones((1, TQ), F32))
    ok = finish_deferred(jnp.int32(NITEM - 1), ok)

    def exact(b):
        row24 = _iota((VR, TQ), 0)

        def item(t, carry):
            h, qs = t // NQS, t % NQS
            par = h % 2
            w = qT[b, qs, pl.ds(5 * (h // 2) + 2 * par, 3)].reshape(VR, TQ)
            w = jnp.where(row24 == jnp.where(par == 1, 0, DH), 0.0, w)

            def pass1(vc, m):
                if b == 1:
                    e0 = P_KB + par * EH + vc * (EH // NQS)
                    kc = jnp.concatenate([pool[e0 + g // NL, :, _lanes(g % NL)] for g in range(TQ // 16)], axis=0)
                else:
                    kc = kh[h, pl.ds(pl.multiple_of(vc * (TQ // 2), TQ // 2), TQ // 2), :]
                s = jnp.dot(pltpu.bitcast(kc, BF16)[:, :VR], w, preferred_element_type=F32)
                sfb[vc] = s
                return jnp.maximum(m, jnp.max(s, axis=0, keepdims=True))

            m = lax.fori_loop(0, NQS, pass1, jnp.full((1, TQ), -jnp.inf, F32))

            def pass2(vc, acc):
                p = _rev8(jnp.exp2(sfb[vc] - m))
                if b == 1:
                    vt = _u2f(jnp.concatenate([pool[P_VB + (par * 3 + t3) * NQS + vc] for t3 in range(3)], axis=0))
                else:
                    vt = vT[h, vc]
                return acc + jnp.dot(vt, p, preferred_element_type=F32)

            acc = lax.fori_loop(0, NQS, pass2, jnp.zeros((VR, TQ), F32))
            l = jnp.where(par == 1, acc[0:1, :], acc[DH:DH + 1, :])
            oT[b, h, qs] = acc * (1.0 / l)
            return carry

        lax.fori_loop(0, H * NQS, item, 0)

    @pl.when(jnp.min(ok) < 0.5)
    def _():
        exact(0)
        exact(1)

    for c in c_wo:
        c.wait()

    def o_copy(qs, b):
        return cp(obuf.at[qs, b], o_hbm.at[pl.ds(qs * TQ, TQ), pl.ds(b * D, D)], osem.at[2 * qs + b])

    for qs in range(NQS):
        for b in range(2):
            parts = []
            for j in range(H // 2):
                e = oT[b, 2 * j, qs]
                o = oT[b, 2 * j + 1, qs]
                parts += [e[0:16], jnp.where(r8 < 4, e[16:24], o[0:8]), o[8:24]]
            ot = jnp.concatenate(parts, axis=0).astype(BF16)
            out = lax.dot_general(ot, wo[b], TN, preferred_element_type=F32)
            obuf[qs, b] = out.astype(BF16)
            o_copy(qs, b).start()
    for qs in range(NQS):
        for b in range(2):
            o_copy(qs, b).wait()


@jax.jit
def pallas_concat_heads__softmax_full_mha__grouped_kv_mqa__prompt_kernel(
    A_x: jax.Array,
    A_wqkv: jax.Array,
    A_wo: jax.Array,
    B_x: jax.Array,
    B_wq: jax.Array,
    B_wk: jax.Array,
    B_wv: jax.Array,
    B_wo: jax.Array,
):
    args = (A_x.reshape(S, D), A_wqkv, A_wo, B_x.reshape(S, D), B_wq, B_wk.T, B_wv.T, B_wo)
    out = pl.pallas_call(
        _kernel,
        in_specs=[pl.BlockSpec(memory_space=pl.ANY)] * 8,
        out_specs=pl.BlockSpec(memory_space=pl.ANY),
        out_shape=jax.ShapeDtypeStruct((S, 2 * D), BF16),
        scratch_shapes=[
            pltpu.VMEM((S, D), BF16),
            pltpu.VMEM((S, D), BF16),
            pltpu.VMEM((D, D), BF16),
            pltpu.VMEM((D, 3 * D), BF16),
            pltpu.VMEM((DH, D), BF16),
            pltpu.VMEM((DH, D), BF16),
            pltpu.VMEM((2, D, D), BF16),
            pltpu.VMEM((NQS, 2, TQ, D), BF16),
            pltpu.VMEM((3 * D, D), BF16),
            pltpu.VMEM((128, D), BF16),
            pltpu.VMEM((H, S // 2, 128), U32),
            pltpu.VMEM((2, NQS, D // 8, 8, TQ), F32),
            pltpu.VMEM((H, NQS, VR, TQ), F32),
            pltpu.VMEM((2, H, NQS, VR, TQ), F32),
            pltpu.VMEM((P_END, 8, TQ), U32),
            pltpu.VMEM((2, H, D), F32),
            pltpu.VMEM((2, NQS, H, 8, TQ), F32),
            pltpu.VMEM((5, S // 2, 128), U32),
            pltpu.VMEM((NQS, TQ, TQ), F32),
            pltpu.SMEM((1,), jnp.int32),
            pltpu.SemaphoreType.DMA((8 + 2 * NQS,)),
            pltpu.SemaphoreType.DMA((2 * NQS,)),
        ],
        compiler_params=pltpu.CompilerParams(vmem_limit_bytes=110 * 1024 * 1024),
        name="attn",
    )(*args)
    return out.reshape(1, S, 2 * D)
```

```python
import jax
import jax.numpy as jnp
from jax import lax
import jax.experimental.pallas as pl
import jax.experimental.pallas.tpu as pltpu

S = 2048
D = 640
H = 32
DH = 20
VR = 24
F32 = jnp.float32
BF16 = jnp.bfloat16
U32 = jnp.uint32
NT = (((1,), (1,)), ((), ()))
TN = (((0,), (0,)), ((), ()))
ONE2 = 0x3F803F80
QSCALE = (DH ** -0.5) * 1.4426950408889634
INFL = 1.0 + 2.0 ** -6
THR = 2.0 ** -24

TQ = 512
CK = 128
NQS = S // TQ
NCH = S // CK
NL = TQ // 128
NITEM = (H // 2) * NQS
NS = 4
NV = [(48, 32, 32, 32)[c % 4] for c in range(NCH)]
SHIFT = (16, 48)
TAIL = 64
GV = max(NV) // 8
EK = -(-GV // NL)
EH = S // 16 // NL
P_QBC = 0
P_PV = P_QBC + NS * (DH + 1)
P_WST = P_PV + NS * NCH * GV
P_KBC = P_WST + NS * 2 * 3
P_KB = P_KBC + NCH * DH * EK
P_VB = P_KB + 2 * EH
P_KA = P_VB + 2 * 3 * NQS
P_VA = P_KA + 2 * EH
P_DEF = P_VA + 2 * 3 * NQS
P_ACC = P_DEF + 16
P_END = P_ACC + 3
AX, BX = 8, 8 + NQS


def _f2u(x):
    return lax.bitcast_convert_type(x, U32)


def _u2f(x):
    return lax.bitcast_convert_type(x, F32)


def _lanes(lt):
    return pl.ds(lt * 128, 128)


def _iota(shape, dim):
    return lax.broadcasted_iota(jnp.int32, shape, dim)


def _rev8(x):
    return jnp.concatenate([x[c * CK + g * 8:c * CK + g * 8 + 8] for c in range(x.shape[0] // CK)
                            for g in range(CK // 8 - 1, -1, -1)], axis=0)


def _gate_at(events, frac, tail=TAIL):
    x = frac * (sum(e.shape[0] // 8 * NL * w for e, w in events) - tail)
    for e, w in events:
        per = e.shape[0] // 8 * NL
        if x < per * w:
            vi = min(int(x / w), per - 1)
            g, lt = (vi // NL) * 8, vi % NL
            return e[g:g + 8, lt * 128:(lt + 1) * 128]
        x -= per * w


def _kernel(ax_hbm, wqkv_hbm, awo_hbm, bx_hbm, bwq_hbm, bwkT_hbm, bwvT_hbm, bwo_hbm,
            o_hbm,
            ax, bx, wka, wsrc, wkT, wvT, wo, obuf,
            wT, wkvT, kh, qT, vT, oT, pool, kmax, mt, kw, sfb, zref, isem, osem):
    zref[0] = 0
    cp = pltpu.make_async_copy

    def x_copy(hbm, buf, base, r):
        rows = pl.ds(pl.multiple_of(r * TQ, TQ), TQ)
        return cp(hbm.at[rows, :], buf.at[rows, :], isem.at[base + r])

    c_wka = [cp(wqkv_hbm.at[:, pl.ds(D, 256)], wka.at[:, pl.ds(0, 256)], isem.at[0]),
             cp(wqkv_hbm.at[:, pl.ds(D + 256, D - 256)], wka.at[:, pl.ds(256, D - 256)], isem.at[8 + 2 * NQS])]
    c_ws = [cp(wqkv_hbm.at[:, pl.ds(0, D)], wsrc.at[:, pl.ds(0, D)], isem.at[1]),
            cp(wqkv_hbm.at[:, pl.ds(2 * D, D)], wsrc.at[:, pl.ds(D, D)], isem.at[2]),
            cp(bwq_hbm, wsrc.at[:, pl.ds(2 * D, D)], isem.at[3])]
    c_small = [cp(bwkT_hbm, wkT, isem.at[4]), cp(bwvT_hbm, wvT, isem.at[5])]
    c_wo = [cp(awo_hbm, wo.at[0], isem.at[6]), cp(bwo_hbm, wo.at[1], isem.at[7])]

    c_wka[0].start()
    x_copy(ax_hbm, ax, AX, 0).start()
    c_wka[1].start()
    for r in range(1, NQS - 1):
        x_copy(ax_hbm, ax, AX, r).start()
    for c in c_ws:
        c.start()
    x_copy(ax_hbm, ax, AX, NQS - 1).start()
    for c in c_small:
        c.start()
    for r in range(NQS):
        x_copy(bx_hbm, bx, BX, r).start()
    for c in c_wo:
        c.start()

    def k_cols(r, w0, w1):
        km = None
        for sub in range(TQ // 256):
            rows = pl.ds(pl.multiple_of(r * TQ, TQ) + sub * 256, 256)
            prow = pl.ds(pl.multiple_of(r * (TQ // 2), TQ // 2) + sub * 128, 128)
            n = (w1 - w0) * 128
            ka = jnp.dot(ax[rows, :], wka[:, pl.ds(w0 * 128, n)], preferred_element_type=F32)
            mx = jnp.max(jnp.abs(ka).reshape(32, 8, n), axis=0)
            km = mx if km is None else jnp.maximum(km, mx)
            ka = _rev8(ka)
            for w in range(w0, w1):
                kw[w, prow, :] = pltpu.bitcast(ka[:, (w - w0) * 128:(w - w0 + 1) * 128].astype(BF16), U32)
        return km

    def k_proj(r, kma):
        x_copy(ax_hbm, ax, AX, r).wait()
        return jnp.maximum(kma, k_cols(r, 0, 5))

    c_wka[0].wait()
    x_copy(ax_hbm, ax, AX, 0).wait()
    km0 = k_cols(0, 0, 2)
    c_wka[1].wait()
    kma = jnp.concatenate([km0, k_cols(0, 2, 5)], axis=1)
    kma = lax.fori_loop(1, NQS - 1, k_proj, kma)
    for c in c_ws:
        c.wait()
    for c in c_small:
        c.wait()
    kma = k_proj(NQS - 1, kma)
    for i in range(15):
        wT[pl.ds(i * 128, 128), :] = wsrc[:, pl.ds(i * 128, 128)].T
    wkvT[...] = jnp.zeros(wkvT.shape, wkvT.dtype)
    wkvT[pl.ds(0, DH), :] = wkT[...]
    wkvT[pl.ds(32, DH), :] = wvT[...]

    hrow, hcol = _iota((H, D), 0), _iota((H, D), 1)
    inhead = jnp.logical_and(hcol >= hrow * DH, hcol < hrow * DH + DH)
    kmax[0] = jnp.where(inhead, jnp.max(kma, axis=0, keepdims=True) * INFL, 0.0)

    def bound(b, r):
        qa = jnp.abs(qT[b, r].reshape(D, TQ))
        bd = jnp.dot(kmax[b], qa, preferred_element_type=F32)
        nb = (-(bd * INFL)).astype(BF16).astype(F32)
        for h in range(H):
            mt[b, r, h] = jnp.broadcast_to(nb[h:h + 1, :], (8, TQ))

    def proj(r, kmb):
        x_copy(bx_hbm, bx, BX, r).wait()
        r0 = pl.multiple_of(r * TQ, TQ)
        row = _iota((VR, TQ), 0)
        xs = (ax[pl.ds(r0, TQ), :], bx[pl.ds(r0, TQ), :])

        lane = _iota((128, 128), 1)
        rw = _iota((VR, 256), 0)
        for sub in range(TQ // 256):
            rows = pl.ds(r0 + sub * 256, 256)
            kvb = lax.dot_general(bx[rows, :], wkvT[...], NT, preferred_element_type=F32)
            kmb = jnp.maximum(kmb, jnp.max(jnp.abs(kvb).reshape(32, 8, 128), axis=0))
            kvb2 = pltpu.roll(kvb, 4, 1)
            k1 = pltpu.bitcast(_rev8(kvb).astype(BF16), U32)
            k2 = pltpu.bitcast(_rev8(kvb2).astype(BF16), U32)
            k1 = jnp.where(lane == DH, jnp.uint32(ONE2), k1)
            k2 = jnp.where(lane == 0, jnp.uint32(ONE2), k2)
            e0 = r * (EH // NQS) + sub * (16 // NL)
            for par, kk in ((0, k1), (1, k2)):
                for t in range(16):
                    pool[P_KB + par * EH + e0 + t // NL, :, _lanes(t % NL)] = kk[t * 8:(t + 1) * 8]
            for cc in range(256 // CK):
                ci = r * (TQ // CK) + sub * (256 // CK) + cc
                gv = NV[sub * (256 // CK) + cc] // 8
                kr = kvb[cc * CK:cc * CK + gv * 8, :].astype(BF16).astype(F32)
                for d in range(DH):
                    kb = _f2u(jnp.broadcast_to(kr[:, d:d + 1], (gv * 8, 128)))
                    for g in range(gv):
                        pool[P_KBC + (ci * EK + g // NL) * DH + d, :, _lanes(g % NL)] = kb[g * 8:(g + 1) * 8]
            v1 = _f2u(jnp.where(rw == DH, 1.0, kvb.T[32:32 + VR, :]))
            v2 = _f2u(jnp.where(rw == 0, 1.0, kvb2.T[32:32 + VR, :]))
            for par, vv in ((0, v1), (1, v2)):
                for t in range(3):
                    pool[P_VB + (par * 3 + t) * NQS + r, :, pl.ds(sub * 256, 256)] = vv[t * 8:(t + 1) * 8]

        def q_proj(b):
            for c in range(5):
                q = lax.dot_general(wT[pl.ds(2 * D * b + c * 128, 128), :], xs[b], NT,
                                    preferred_element_type=F32)
                q = (q * QSCALE).astype(BF16).astype(F32)
                qT[b, r, pl.ds(c * 16, 16)] = q.reshape(16, 8, TQ)

        def v_proj(c):
            v = lax.dot_general(wT[pl.ds(D + c * 160, 160), :], xs[0], NT, preferred_element_type=F32)
            for j in range(4):
                e = v[40 * j:40 * j + VR, :]
                o = v[40 * j + 16:40 * j + 16 + VR, :]
                vT[c * 8 + 2 * j, r] = jnp.where(row == DH, 1.0, e)
                vT[c * 8 + 2 * j + 1, r] = jnp.where(row == 0, 1.0, o)

        q_proj(0)
        v_proj(0)
        v_proj(1)
        bound(0, r)
        v_proj(2)
        v_proj(3)
        q_proj(1)
        lane = _iota((64, 128), 1)
        for sub in range(TQ // 128):
            prow = pl.ds(pl.multiple_of(r * (TQ // 2), TQ // 2) + sub * 64, 64)
            ws = [kw[w, prow, :] for w in range(5)]
            for h in range(H):
                w, lo = divmod(DH * h, 128)
                src = ws[w] if lo + DH <= 128 else jnp.where(lane >= 64, ws[w], ws[w + 1])
                off = 4 * (h % 2)
                sh = (128 - lo + off) % 128
                if sh:
                    src = pltpu.roll(src, sh, 1)
                keep = (lane >= off) if off else (lane < DH)
                fill = jnp.where(lane == (0 if off else DH), jnp.uint32(ONE2), jnp.uint32(0))
                kh[h, prow, :] = jnp.where(keep, src, fill)
        return kmb

    kmb = lax.fori_loop(0, NQS, proj, jnp.zeros((8, 128), F32))

    trow, tcol = _iota((128, D), 0), _iota((128, D), 1)
    sel = jnp.zeros((128, D), F32)
    for h in range(H):
        sel = jnp.where(jnp.logical_and(tcol - h * DH == trow, trow < DH), 1.0, sel)
    kmb_up = (jnp.max(kmb, axis=0, keepdims=True) * INFL).astype(BF16).astype(F32)
    kmb_up = jnp.where(_iota((8, 128), 1) < DH, jnp.broadcast_to(kmb_up, (8, 128)), 0.0)
    kmb_t = jnp.dot(kmb_up, sel, preferred_element_type=F32)[0:1, :]
    kmax[1] = jnp.where(inhead, kmb_t, 0.0)
    bound(1, 0)
    bound(1, 1)

    r8 = _iota((8, TQ), 0)

    def q_window(b, it, par):
        j, qs = it // NQS, it % NQS
        w = qT[b, qs, pl.ds(5 * j + 2 * par, 3)]
        nb = mt[b, qs, 2 * j + par]
        if par:
            return jnp.concatenate([jnp.where(r8 == 0, nb, w[0]), w[1], w[2]], axis=0)
        return jnp.concatenate([w[0], w[1], jnp.where(r8 == 4, nb, w[2])], axis=0)

    def build_qbc(it, par, slot, events):
        wb = q_window(1, it, par)
        never = zref[0] != 0
        n = 0
        for t in range(3):
            for lt in range(NL):
                blk = wb[t * 8:(t + 1) * 8, lt * 128:(lt + 1) * 128]
                if events is not None:
                    blk = jnp.where(never, _gate_at(events, (n + 0.5) / (3 * NL + 1)), blk)
                n += 1
                for rr in range(8):
                    d = t * 8 + rr - 4 * par
                    if t * 8 + rr == (0 if par else DH):
                        d = DH
                    elif not 0 <= d < DH:
                        continue
                    v = jnp.broadcast_to(blk[rr:rr + 1, :], (8, 128))
                    pool[P_QBC + slot * (DH + 1) + d, :, _lanes(lt)] = _f2u(v)

    def vpu_scores(pair, chunks, events, tail):
        never = zref[0] != 0
        strips = [(c, g) for c in chunks for g in range(NV[c] // 8)]
        nsteps = len(strips) * DH
        for jb, (c, g) in enumerate(strips):
            gates = jnp.concatenate([_gate_at(events, (jb * DH + d) / nsteps, tail) for d in range(DH)], axis=0)
            kb = _u2f(pool[pl.ds(P_KBC + (c * EK + g // NL) * DH, DH), :, _lanes(g % NL)])
            kb = jnp.where(never, gates.reshape(DH, 8, 128), kb)
            kb = jnp.concatenate([kb] * NL, axis=2)
            for slot in (2 * pair, 2 * pair + 1):
                qi = P_QBC + slot * (DH + 1)
                s = jnp.sum(kb * _u2f(pool[pl.ds(qi, DH)]), axis=0) + _u2f(pool[qi + DH])
                pool[P_PV + (slot * NCH + c) * GV + g] = _f2u(jnp.exp2(s))

    def pool_vt(base, par, c):
        vc, vo = divmod(c * CK, TQ)
        return _u2f(jnp.concatenate([pool[base + (par * 3 + t) * NQS + vc, :, pl.ds(vo, CK)]
                                     for t in range(3)], axis=0))

    def finish(acc, b, it, par, ok):
        lr = 0 if par else DH
        l = acc[lr:lr + 1, :]
        oT[b, 2 * (it // NQS) + par, it % NQS] = acc * (1.0 / l)
        return jnp.where(jnp.logical_and(l >= THR, l <= 4.0 * S), ok, 0.0)

    class Stage:
        def __init__(self, b, slot, it, events):
            self.b, self.par, self.slot, self.it, self.events = b, slot % 2, slot, it, events
            self.nv = NV if b == 1 else [0] * NCH
            self.head = 2 * (it // NQS) + self.par
            self.groups = [c * 8 + g for c in range(NCH) for g in range((CK - self.nv[c]) // 16)]
            self.pos = 0
            self.p8 = {}
            self.last = False
            self.w0 = P_WST + (slot * 2 + b) * 3
            pool[pl.ds(self.w0, 3)] = _f2u(q_window(b, it, self.par)).reshape(3, 8, TQ)

        def qk(self, c):
            end = sum((CK - self.nv[i]) // 16 for i in range(c + 1)) + SHIFT[self.b] // 16
            gs = self.groups[self.pos:min(end, len(self.groups))]
            self.pos += len(gs)
            if self.b == 1 or self.slot >= 2:
                base = (P_KB if self.b == 1 else P_KA) + self.par * EH
                parts = [pool[base + g // NL, :, _lanes(g % NL)] for g in gs]
            else:
                parts = [kh[self.head, pl.ds(g * 8, 8), :] for g in gs]
                for g, pt in zip(gs, parts):
                    pool[P_KA + self.par * EH + g // NL, :, _lanes(g % NL)] = pt
            kc = pltpu.bitcast(jnp.concatenate(parts, axis=0) if len(parts) > 1 else parts[0], BF16)
            wq = _u2f(pool[pl.ds(self.w0, 3)]).reshape(VR, TQ)
            s = jnp.dot(kc[:, :VR], wq, preferred_element_type=F32)
            nm = S - sum(self.nv)
            self.events.append((s, ((nm + VR * NCH) / nm) / ((CK + VR) / CK)))
            p = jnp.exp2(s)
            for i, g in enumerate(gs):
                self.p8[2 * g] = p[16 * i:16 * i + 8]
                self.p8[2 * g + 1] = p[16 * i + 8:16 * i + 16]

        def pv(self, c, ok):
            b, par, nv = self.b, self.par, self.nv[c]
            parts = []
            if nv:
                parts.append(_u2f(pool[pl.ds(P_PV + (self.slot * NCH + c) * GV, nv // 8)]).reshape(nv, TQ))
            for g in range(nv // 8, CK // 8):
                parts.append(self.p8.pop(c * 16 + 15 - g))
            p = jnp.concatenate(parts, axis=0)
            if self.last and c == NCH - 1:
                pool[pl.ds(P_DEF, 16)] = _f2u(p).reshape(16, 8, TQ)
                return ok
            if b == 1 or self.slot >= 2:
                vt = pool_vt(P_VB if b == 1 else P_VA, par, c)
            else:
                vc, vo = divmod(c * CK, TQ)
                vt = vT[self.head, vc, :, pl.ds(vo, CK)]
                for t in range(3):
                    pool[P_VA + (par * 3 + t) * NQS + vc, :, pl.ds(vo, CK)] = _f2u(vt[t * 8:(t + 1) * 8])
            acc = jnp.dot(vt, p, preferred_element_type=F32)
            if c > 0:
                acc = _u2f(pool[pl.ds(P_ACC, 3)]).reshape(VR, TQ) + acc
            if c < NCH - 1:
                pool[pl.ds(P_ACC, 3)] = _f2u(acc).reshape(3, 8, TQ)
                return ok
            return finish(acc, b, self.it, par, ok)

    def finish_deferred(it, ok):
        acc = _u2f(pool[pl.ds(P_ACC, 3)]).reshape(VR, TQ)
        p = _u2f(pool[pl.ds(P_DEF, 16)]).reshape(CK, TQ)
        acc = acc + jnp.dot(pool_vt(P_VA, 1, NCH - 1), p, preferred_element_type=F32)
        return finish(acc, 0, it, 1, ok)

    def body(i, ok):
        ok = finish_deferred(jnp.maximum(i, 1) * 2 - 1, ok)
        evs = [[] for _ in range(NS)]
        st = []
        for k in range(NS):
            st += [Stage(1, k, i * 2 + k // 2, evs[k]), Stage(0, k, i * 2 + k // 2, evs[k])]
        st[-1].last = True
        slots = [(s, c) for s in st for c in range(NCH)]
        for n in range(len(slots) + 1):
            if n == 3 * NCH:
                vpu_scores(1, range(NCH // 2, NCH), evs[0], 0)
            if n < len(slots):
                slots[n][0].qk(slots[n][1])
                if slots[n][1] == NCH - 1 and n + 1 < len(slots):
                    slots[n + 1][0].qk(-1)
            if n >= 1:
                s, c = slots[n - 1]
                ok = s.pv(c, ok)
        itn = jnp.minimum(i + 1, NITEM // 2 - 1) * 2
        h0 = len(evs[0]) // 2
        build_qbc(itn, 0, 0, evs[0][:h0])
        build_qbc(itn, 1, 1, evs[0][h0:])
        vpu_scores(0, range(NCH), evs[1] + evs[2], 0)
        build_qbc(itn + 1, 0, 2, evs[1])
        build_qbc(itn + 1, 1, 3, evs[2])
        vpu_scores(1, range(NCH // 2), evs[3], TAIL)
        return ok

    for k in range(NS):
        if k in (1, 2):
            bound(1, k + 1)
        wq = q_window(1, k // 2, k % 2)
        base = P_KB + (k % 2) * EH
        for c4 in range(NCH // 4 if k < 2 else NCH // 8):
            gl = [c * 8 + 8 - NV[c] // 16 + i for c in range(c4 * 4, c4 * 4 + 4) for i in range(NV[c] // 16)]
            kc = jnp.concatenate([pool[base + g // NL, :, _lanes(g % NL)] for g in gl], axis=0)
            pp = _f2u(jnp.exp2(jnp.dot(pltpu.bitcast(kc, BF16)[:, :VR], wq, preferred_element_type=F32)))
            for i, g in enumerate(gl):
                for hf in range(2):
                    c, st8 = g // 8, (g % 8) * 2 + hf
                    pool[P_PV + (k * NCH + c) * GV + 15 - st8] = pp[16 * i + 8 * hf:16 * i + 8 * hf + 8]
    build_qbc(1, 0, 2, None)
    build_qbc(1, 1, 3, None)
    pool[pl.ds(P_DEF, 19)] = _f2u(jnp.ones((19, 8, TQ), F32))
    for t in range(3):
        pool[P_VA + (3 + t) * NQS + NQS - 1] = jnp.zeros((8, TQ), U32)

    ok = lax.fori_loop(0, NITEM // 2, body, jnp.ones((1, TQ), F32))
    ok = finish_deferred(jnp.int32(NITEM - 1), ok)

    def exact(b):
        row24 = _iota((VR, TQ), 0)

        def item(t, carry):
            h, qs = t // NQS, t % NQS
            par = h % 2
            w = qT[b, qs, pl.ds(5 * (h // 2) + 2 * par, 3)].reshape(VR, TQ)
            w = jnp.where(row24 == jnp.where(par == 1, 0, DH), 0.0, w)

            def pass1(vc, m):
                if b == 1:
                    e0 = P_KB + par * EH + vc * (EH // NQS)
                    kc = jnp.concatenate([pool[e0 + g // NL, :, _lanes(g % NL)] for g in range(TQ // 16)], axis=0)
                else:
                    kc = kh[h, pl.ds(pl.multiple_of(vc * (TQ // 2), TQ // 2), TQ // 2), :]
                s = jnp.dot(pltpu.bitcast(kc, BF16)[:, :VR], w, preferred_element_type=F32)
                sfb[vc] = s
                return jnp.maximum(m, jnp.max(s, axis=0, keepdims=True))

            m = lax.fori_loop(0, NQS, pass1, jnp.full((1, TQ), -jnp.inf, F32))

            def pass2(vc, acc):
                p = _rev8(jnp.exp2(sfb[vc] - m))
                if b == 1:
                    vt = _u2f(jnp.concatenate([pool[P_VB + (par * 3 + t3) * NQS + vc] for t3 in range(3)], axis=0))
                else:
                    vt = vT[h, vc]
                return acc + jnp.dot(vt, p, preferred_element_type=F32)

            acc = lax.fori_loop(0, NQS, pass2, jnp.zeros((VR, TQ), F32))
            l = jnp.where(par == 1, acc[0:1, :], acc[DH:DH + 1, :])
            oT[b, h, qs] = acc * (1.0 / l)
            return carry

        lax.fori_loop(0, H * NQS, item, 0)

    @pl.when(jnp.min(ok) < 0.5)
    def _():
        exact(0)
        exact(1)

    for c in c_wo:
        c.wait()

    pieces = [(qs, b, 0, TQ) for qs in range(NQS) for b in range(2)][:-1]
    pieces += [(NQS - 1, 1, 0, 384), (NQS - 1, 1, 384, 128)]

    def o_copy(n):
        qs, b, r0, nr = pieces[n]
        return cp(obuf.at[qs, b, pl.ds(r0, nr), :], o_hbm.at[pl.ds(qs * TQ + r0, nr), pl.ds(b * D, D)], osem.at[n])

    for n, (qs, b, r0, nr) in enumerate(pieces):
        parts = []
        for j in range(H // 2):
            e = oT[b, 2 * j, qs, :, pl.ds(r0, nr)]
            o = oT[b, 2 * j + 1, qs, :, pl.ds(r0, nr)]
            parts += [e[0:16], jnp.where(_iota((8, nr), 0) < 4, e[16:24], o[0:8]), o[8:24]]
        ot = jnp.concatenate(parts, axis=0).astype(BF16)
        out = lax.dot_general(ot, wo[b], TN, preferred_element_type=F32)
        obuf[qs, b, pl.ds(r0, nr), :] = out.astype(BF16)
        o_copy(n).start()
    for n in range(len(pieces)):
        o_copy(n).wait()


@jax.jit
def pallas_concat_heads__softmax_full_mha__grouped_kv_mqa__prompt_kernel(
    A_x: jax.Array,
    A_wqkv: jax.Array,
    A_wo: jax.Array,
    B_x: jax.Array,
    B_wq: jax.Array,
    B_wk: jax.Array,
    B_wv: jax.Array,
    B_wo: jax.Array,
):
    args = (A_x.reshape(S, D), A_wqkv, A_wo, B_x.reshape(S, D), B_wq, B_wk.T, B_wv.T, B_wo)
    out = pl.pallas_call(
        _kernel,
        in_specs=[pl.BlockSpec(memory_space=pl.ANY)] * 8,
        out_specs=pl.BlockSpec(memory_space=pl.ANY),
        out_shape=jax.ShapeDtypeStruct((S, 2 * D), BF16),
        scratch_shapes=[
            pltpu.VMEM((S, D), BF16),
            pltpu.VMEM((S, D), BF16),
            pltpu.VMEM((D, D), BF16),
            pltpu.VMEM((D, 3 * D), BF16),
            pltpu.VMEM((DH, D), BF16),
            pltpu.VMEM((DH, D), BF16),
            pltpu.VMEM((2, D, D), BF16),
            pltpu.VMEM((NQS, 2, TQ, D), BF16),
            pltpu.VMEM((3 * D, D), BF16),
            pltpu.VMEM((128, D), BF16),
            pltpu.VMEM((H, S // 2, 128), U32),
            pltpu.VMEM((2, NQS, D // 8, 8, TQ), F32),
            pltpu.VMEM((H, NQS, VR, TQ), F32),
            pltpu.VMEM((2, H, NQS, VR, TQ), F32),
            pltpu.VMEM((P_END, 8, TQ), U32),
            pltpu.VMEM((2, H, D), F32),
            pltpu.VMEM((2, NQS, H, 8, TQ), F32),
            pltpu.VMEM((5, S // 2, 128), U32),
            pltpu.VMEM((NQS, TQ, TQ), F32),
            pltpu.SMEM((1,), jnp.int32),
            pltpu.SemaphoreType.DMA((9 + 2 * NQS,)),
            pltpu.SemaphoreType.DMA((2 * NQS + 1,)),
        ],
        compiler_params=pltpu.CompilerParams(vmem_limit_bytes=110 * 1024 * 1024),
        name="attn",
    )(*args)
    return out.reshape(1, S, 2 * D)
```
